```python
import jax
import jax.numpy as jnp

def _softmax(x, axis=-1):
    return jax.nn.softmax(x, axis=axis)
def _gelu(x):
    return jax.nn.gelu(x, approximate=True)
def _silu(x):
    return jax.nn.silu(x)
def _sigmoid(x):
    return jax.nn.sigmoid(x)
def _layernorm(x, axis=-1, eps=1e-5):
    m = jnp.mean(x, axis=axis, keepdims=True)
    v = jnp.var(x, axis=axis, keepdims=True)
    return (x - m) / jnp.sqrt(v + eps)
def _scatter_add(tgt, idx, src, axis=0):
    return tgt.at[idx].add(src)
def _segment_sum(src, seg, n):
    return jax.ops.segment_sum(src, seg, n)
class _Rng:
    def __init__(self, key):
        self._k = key
    def _next(self):
        self._k, sub = jax.random.split(self._k)
        return sub
    def normal(self, shape):
        return jax.random.normal(self._next(), shape, dtype=jnp.bfloat16)
    def randint(self, lo, hi, shape):
        return jax.random.randint(self._next(), shape, lo, hi, dtype=jnp.int32)
    def uniform(self, shape, lo=0.0, hi=1.0):
        return jax.random.uniform(self._next(), shape, jnp.bfloat16, lo, hi)
    def permutation(self, n):
        return jax.random.permutation(self._next(), n)


kernel_name = 'standalone__seq2seq_rnn_t_joint__speech'

def _fwd_setup_inputs():
    _rng = _Rng(jax.random.key(int.from_bytes(__import__("os").urandom(4), "little")))
    _w = (lambda a: (lambda t: t.astype(jnp.bfloat16) if jnp.issubdtype(t.dtype, jnp.floating) else t)(jnp.asarray(a)))
    B, T, D, K = 2, 1000, 512, 5
    U = 8
    sc = (1.0 / (K * D)) ** 0.5
    sd = (1.0 / D) ** 0.5
    return {
        "x": _w((lambda *s: _rng.normal(s) * 0.05)(B, T, D) * 0.5),
        "w1": _w((lambda *s: _rng.normal(s) * 0.05)(K, D, D) * sc),
        "w2": _w((lambda *s: _rng.normal(s) * 0.05)(K, D, D) * sc),
        "g": _w((lambda *s: _rng.normal(s) * 0.05)(B, U, D) * 0.5),
        "w_f": _w((lambda *s: _rng.normal(s) * 0.05)(D, D) * sd),
        "w_g": _w((lambda *s: _rng.normal(s) * 0.05)(D, D) * sd),
        "w_o": _w((lambda *s: _rng.normal(s) * 0.05)(D, D) * sd),
    }

def _fwd_reference(x, w1, w2, g, w_f, w_g, w_o):
    B, T, D = x.shape
    K = w1.shape[0]
    pad = K // 2
    xp = jnp.pad(x, ((0,0),(pad,pad),(0,0)))
    h = jnp.zeros_like(x)
    for i in range(K):
        h = h + jnp.einsum("btc,cd->btd", xp[:, i:i+T, :], w1[i])
    h = _gelu(h)[:, ::2, :]
    T1 = h.shape[1]
    hp = jnp.pad(h, ((0,0),(pad,pad),(0,0)))
    f = jnp.zeros_like(h)
    for i in range(K):
        f = f + jnp.einsum("btc,cd->btd", hp[:, i:i+T1, :], w2[i])
    f = _gelu(f)[:, ::2, :]
    fe = jnp.einsum("btd,de->bte", f, w_f)
    ge = jnp.einsum("bud,de->bue", g, w_g)
    j = jnp.tanh(fe[:, :, None, :] + ge[:, None, :, :])
    return jnp.einsum("btud,dv->btuv", j, w_o)


def setup_inputs():
    _inp = _fwd_setup_inputs()
    _gk = jax.random.fold_in(jax.random.key(int.from_bytes(__import__("os").urandom(4), "little")), 2**31 - 1)
    _shapes = [[2, 250, 8, 512]]
    _dtypes = ['bfloat16']
    _gks = jax.random.split(_gk, len(_shapes))
    _gs = [jax.random.normal(k, s, dtype=jnp.dtype(d)) * 0.05 for k, s, d in zip(_gks, _shapes, _dtypes)]
    _inp["grad_out"] = _gs[0]
    return _inp

def reference(x, w1, w2, g, w_f, w_g, w_o, grad_out):
    _const = dict()
    def _f(*_d):
        return _fwd_reference(**{'x': _d[0], 'w1': _d[1], 'w2': _d[2], 'g': _d[3], 'w_f': _d[4], 'w_g': _d[5], 'w_o': _d[6], **_const})
    _out, _vjp = jax.vjp(_f, x, w1, w2, g, w_f, w_g, w_o)
    _grads = _vjp(grad_out)
    _out0 = jnp.asarray(_out)
    return (_out0, *[jnp.asarray(_g) for _g in _grads])
```

```python
import math

import jax
import jax.numpy as jnp
from jax import lax
import jax.experimental.pallas as pl
import jax.experimental.pallas.tpu as pltpu

CFG = dict(GO_CH=(256, 256, 512, 992, 992, 992), JCH=(64, 61), XC=512, flags={})

F32, BF16, I32 = jnp.float32, jnp.bfloat16, jnp.int32
B, T, D, U = 2, 1000, 512, 8
NT = T // 8
NP = 128
R = B * NP
JR = B * NT * 2 * U
LC = D // 128
XROWS = 16 + 8 * NP + 16

PA2, PB2 = 0.5, 2.0
PA, PB = math.sqrt(PA2), math.sqrt(PB2)
IA, IB = 1.0 / (2 * PA2 * (PA2 - PB2)), 1.0 / (2 * PB2 * (PB2 - PA2))
GC = math.sqrt(2.0 / math.pi)
GK = 0.044715


def _dot(a, b):
    return lax.dot_general(a, b, (((1,), (0,)), ((), ())), preferred_element_type=F32)


def _dot_nt(a, b):
    return lax.dot_general(a, b, (((1,), (1,)), ((), ())), preferred_element_type=F32)


def _dot_tn(a, b):
    return lax.dot_general(a, b, (((0,), (0,)), ((), ())), preferred_element_type=F32)


def _gelu_and_grad(x):
    x2 = x * x
    t = jnp.tanh(x * (GC + (GC * GK) * x2))
    cdf = 0.5 + 0.5 * t
    y = x * cdf
    return y, cdf + y * (1.0 - t) * (GC + (3.0 * GC * GK) * x2)


def _prev(v):
    return pltpu.roll(v, 1, 0)


def _next(v):
    return pltpu.roll(v, v.shape[0] - 1, 0)


def _bf16_bits(v):
    return lax.bitcast_convert_type(v.astype(BF16).astype(F32), I32)


def _sum_sublanes(v):
    m, c = v.shape[0] // 8, v.shape[2]
    sub = lax.broadcasted_iota(I32, (m, 8, c), 1)
    v = v.reshape(m, 8, 8, c)
    parts = [v[:, i] for i in range(8)]
    k = 1
    while len(parts) > 1:
        hi = (sub & k) != 0
        parts = [jnp.where(hi, q, p) + pltpu.roll(jnp.where(hi, p, q), k, 1)
                 for p, q in zip(parts[0::2], parts[1::2])]
        k *= 2
    return parts[0].reshape(8 * m, c)


def _kernel(x_h, w1_h, w2_h, g_h, wf_h, wg_h, wo_h, go_h,
            out_h, dx_h, dw1_h, dw2_h, dg_h, dwf_h, dwg_h, dwo_h,
            xb, wt1, wt2, wr, g_v, wf, wg, wo, go,
            dj, xt1, xt2, gp1, gp2, f_v, fe, j_v, dfe, dm2, dm1,
            out_v, dxb, dw1_v, dw2_v, dg_v, dwf_v, dwg_v, dwo_v, sem):
    n_sem = [0]

    def copy(src, dst):
        cp = pltpu.make_async_copy(src, dst, sem.at[n_sem[0]])
        n_sem[0] += 1
        cp.start()
        return cp

    def blk(i, n=1):
        return slice(i * D, (i + n) * D)

    def lanes(c, n=128):
        return slice(c * n, (c + 1) * n)

    cp_wo = copy(wo_h, wo)
    go_rows, r0 = [], 0
    for n in CFG["GO_CH"]:
        go_rows.append(slice(r0, r0 + n))
        r0 += n
    cp_go = [copy(go_h.at[s], go.at[s]) for s in go_rows]
    cp_w1 = [copy(w1_h.at[0], wt1.at[blk(0)]), copy(w1_h.at[1], wt1.at[blk(1)]),
             copy(w1_h.at[4], wt1.at[blk(10)]), copy(w1_h.at[2:4], wr.at[0:2])]
    cp_x = [copy(x_h.at[:, :, lanes(c)], xb.at[c, :, 16:16 + T]) for c in range(LC)]
    cp_w2 = [copy(w2_h.at[0], wt2.at[blk(0)]), copy(w2_h.at[1], wt2.at[blk(1)]),
             copy(w2_h.at[4], wt2.at[blk(5)]), copy(w2_h.at[3], wt2.at[blk(6)]),
             copy(w2_h.at[2], wr.at[2])]
    cp_rest = [copy(wf_h, wf), copy(wg_h, wg), copy(g_h, g_v)]

    cp_wo.wait()
    for cp, s in zip(cp_go, go_rows):
        cp.wait()
        dj[s, :] = _dot_nt(go[s, :], wo[...])

    for cp in cp_w1:
        cp.wait()
    g0, h0, g2 = (wt1[blk(i), :].astype(F32) for i in (0, 1, 10))
    g1, h1 = wr[0].astype(F32), wr[1].astype(F32)
    for i, p, p2 in ((2, PA, PA2), (6, PB, PB2)):
        ev, od, oo = g0 + p2 * g2, p * g1, p * h1
        wt1[blk(i), :] = (ev + od).astype(BF16)
        wt1[blk(i + 1), :] = (h0 + oo).astype(BF16)
        wt1[blk(i + 2), :] = (ev - od).astype(BF16)
        wt1[blk(i + 3), :] = (h0 - oo).astype(BF16)

    for cp in cp_x:
        cp.wait()
    xw = xb.bitcast(I32)
    tail = slice((16 + T) // 2 - 4, XROWS // 2)
    for c in range(LC):
        for b in range(B):
            xw[c, b, 0:8, :] = jnp.zeros((8, 128), I32)
            ntail = tail.stop - tail.start
            keep = lax.broadcasted_iota(I32, (ntail, 128), 0) < 4
            xw[c, b, tail, :] = jnp.where(keep, xw[c, b, tail, :], 0)
            words = [xw[c, b, pl.ds(7 + k, NP, stride=4), :] for k in range(6)]
            for ph in range(2):
                if ph == 0:
                    d = [lax.bitcast_convert_type(w << 16, F32) for w in words]
                else:
                    d = [lax.bitcast_convert_type(w & -65536, F32) for w in words[:5]]

                def put(i, v):
                    xt1[b * NP:(b + 1) * NP, i * D + c * 128:i * D + (c + 1) * 128] = v.astype(BF16)

                put(ph, d[0] - (PA2 + PB2) * d[2] + d[4])
                for i, p, q2 in ((2, PA, PB2), (6, PB, PA2)):
                    ev, od = d[4] - q2 * d[2], p * (d[3] - q2 * d[1])
                    put(i + ph, ev + od)
                    put(i + 2 + ph, ev - od)
                if ph == 0:
                    put(10, d[1] - (PA2 + PB2) * d[3] + d[5])

    for cp in cp_w2:
        cp.wait()
    ev = wt2[blk(0), :].astype(F32) + wt2[blk(5), :].astype(F32)
    od = wr[2].astype(F32)
    wt2[blk(2), :] = (0.5 * (ev + od)).astype(BF16)
    wt2[blk(3), :] = (wt2[blk(1), :].astype(F32) + wt2[blk(6), :].astype(F32)).astype(BF16)
    wt2[blk(4), :] = (0.5 * (ev - od)).astype(BF16)

    XC = CFG["XC"]
    P1 = ((0, 2), (2, 2), (4, 2), (6, 2), (8, 2), (10, 1))
    P2 = ((0, 2), (2, 2), (4, 1), (5, 2))
    valid = (lax.broadcasted_iota(I32, (R, XC), 0) & (NP - 1)) < NT
    for c in range(D // XC):
        cs = lanes(c, XC)
        m0, ma, mna, mb, mnb, mi = (_dot(xt1[:, blk(*p)], wt1[blk(*p), cs]) for p in P1)
        sa, da, sb, db = ma + mna, ma - mna, mb + mnb, mb - mnb
        pre = (m0 + IA * sa + IB * sb, (IA * PA) * da + (IB * PB) * db,
               (IA * PA2) * sa + (IB * PB2) * sb, (IA * PA * PA2) * da + (IB * PB * PB2) * db + mi)
        h = []
        for q in range(4):
            y, gp = _gelu_and_grad(pre[q])
            h.append(jnp.where(valid, y, 0.0))
            gp1[q, :, cs] = jnp.where(valid, gp, 0.0)
        e0, e1, e2, e3 = _prev(h[2]), h[0], h[2], _next(h[0])
        o0, o1, o2 = _prev(h[3]), h[1], h[3]
        for i, v in enumerate((e0 - e2, o0 - o1, e1 + e2, o1, e2 - e1, e3 - e1, o2 - o1)):
            xt2[:, i * D + c * XC:i * D + (c + 1) * XC] = v.astype(BF16)

    for c in range(D // XC):
        cs = lanes(c, XC)
        m0, m1, mn1, mi = (_dot(xt2[:, blk(*p)], wt2[blk(*p), cs]) for p in P2)
        for q, pre in enumerate((m0 + m1 + mn1, m1 - mn1 + mi)):
            y, gp = _gelu_and_grad(pre)
            f_v[q * R:(q + 1) * R, cs] = y.astype(BF16)
            gp2[q, :, cs] = gp

    for cp in cp_rest:
        cp.wait()
    fe[...] = _dot(f_v[...], wf[...])
    ge = _dot(g_v[...], wg[...])

    cp_out, dwo, dge = [], None, []
    for b in range(B):
        n0, dge_b = 0, None
        for n in CFG["JCH"]:
            rows = slice((b * NT + n0) * 16, (b * NT + n0 + n) * 16)
            npad = -(-n // 8) * 8
            z = [fe[q * R + b * NP + n0:q * R + b * NP + n0 + npad, :][:, None, :]
                 + ge[b * U:(b + 1) * U][None] for q in range(2)]
            j = jnp.tanh(jnp.stack(z, axis=1)[:n])
            dz = dj[rows, :].reshape(n, 2, U, D) * (1.0 - j * j)
            j_v[rows, :] = j.reshape(n * 16, D).astype(BF16)
            s = jnp.sum(dz.reshape(2 * n, U, D), axis=0)
            dge_b = s if dge_b is None else dge_b + s
            if npad > n:
                dz = jnp.concatenate([dz, jnp.zeros((npad - n, 2, U, D), F32)], axis=0)
            for q in range(2):
                dfe[q * R + b * NP + n0:q * R + b * NP + n0 + npad, :] = (
                    _sum_sublanes(dz[:, q]).astype(BF16))
            part = _dot_tn(j_v[rows, :], go[rows, :])
            dwo = part if dwo is None else dwo + part
            out_v[rows, :] = _dot(j_v[rows, :], wo[...]).astype(BF16)
            cp_out.append(copy(out_v.at[rows], out_h.at[rows]))
            n0 += n
        dge.append(dge_b)
    dwo_v[...] = dwo.astype(BF16)
    cp_out.append(copy(dwo_v, dwo_h))

    dge = jnp.concatenate(dge, axis=0).astype(BF16)
    dg_v[...] = _dot_nt(dge, wg[...]).astype(BF16)
    dwg_v[...] = _dot_tn(g_v[...], dge).astype(BF16)
    df = _dot_nt(dfe[...], wf[...])
    dy0, dy1 = df[:R] * gp2[0], df[R:] * gp2[1]
    for i, v in enumerate((dy0, dy0 + dy1, dy0 - dy1, dy1)):
        dm2[i] = v.astype(BF16)
    dwf_v[...] = _dot_tn(f_v[...], dfe[...]).astype(BF16)
    cp_out += [copy(dg_v, dg_h), copy(dwg_v, dwg_h), copy(dwf_v, dwf_h)]

    for c in range(D // XC):
        cs = lanes(c, XC)

        def back2(p, i):
            return _dot_nt(dm2[p], wt2[i * D + c * XC:i * D + (c + 1) * XC, :])

        re0, ro0, re1, ro1, ren, rei, roi = (
            back2(p, i) for i, p in enumerate((0, 0, 1, 1, 2, 3, 3)))
        dh = (re1 - ren - rei + _prev(rei), ro1 - ro0 - roi,
              re1 + ren - re0 + _next(re0), roi + _next(ro0))
        dy = [dh[q] * gp1[q, :, cs] for q in range(4)]
        dm1[0, :, cs] = dy[0].astype(BF16)
        dm1[5, :, cs] = dy[3].astype(BF16)
        for i, p, p2, inv in ((1, PA, PA2, IA), (3, PB, PB2, IB)):
            ev = inv * dy[0] + (inv * p2) * dy[2]
            od = (inv * p) * dy[1] + (inv * p * p2) * dy[3]
            dm1[i, :, cs] = (ev + od).astype(BF16)
            dm1[i + 1, :, cs] = (ev - od).astype(BF16)

    qe0, qo0, qe1, qo1, qen, qei, qoi = (
        _dot_tn(xt2[:, blk(i)], dm2[p]) for i, p in enumerate((0, 0, 1, 1, 2, 3, 3)))
    sm, df_ = 0.5 * (qe1 + qen), 0.5 * (qe1 - qen)
    for i, v in enumerate((qe0 + sm, qo0 + qo1, df_, qo1 + qoi, sm + qei)):
        dw2_v[i] = v.astype(BF16)
    cp_out.append(copy(dw2_v, dw2_h))

    for ph in range(2):
        q0, qa, qna, qb, qnb = (_dot_tn(xt1[:, blk(2 * p + ph)], dm1[p]) for p in range(5))
        sa, sb = qa + qna, qb + qnb
        dw1_v[ph] = (q0 + sa + sb).astype(BF16)
        dw1_v[2 + ph] = (PA * (qa - qna) + PB * (qb - qnb)).astype(BF16)
        if ph == 0:
            dw1_v[4] = (PA2 * sa + PB2 * sb + _dot_tn(xt1[:, blk(10)], dm1[5])).astype(BF16)
    cp_out.append(copy(dw1_v, dw1_h))

    dxw = dxb.bitcast(I32)
    for c in range(D // XC):
        res = []
        for ph in range(2):
            def back1(p, i):
                return _dot_nt(dm1[p], wt1[i * D + c * XC:i * D + (c + 1) * XC, :])

            r0, ra, rna, rb, rnb = (back1(p, 2 * p + ph) for p in range(5))
            sa, da, sb, db = ra + rna, ra - rna, rb + rnb, rb - rnb
            d1 = (-PA * PB2) * da - (PB * PA2) * db
            d2 = (-(PA2 + PB2)) * r0 - PB2 * sa - PA2 * sb
            d3 = PA * da + PB * db
            d4 = r0 + sa + sb + _next(r0)
            if ph == 0:
                ri = back1(5, 10)
                d1 = d1 + ri + _prev(ri)
                d3 = d3 - (PA2 + PB2) * ri
            res.append((d1, d2, d3, d4))
        for q in range(4):
            word = lax.shift_right_logical(_bf16_bits(res[0][q]), 16) | _bf16_bits(res[1][q])
            for cc in range(XC // 128):
                for b in range(B):
                    dxw[c * (XC // 128) + cc, b, pl.ds(q, NP, stride=4), :] = (
                        word[b * NP:(b + 1) * NP, lanes(cc)])
        for cc in range(c * (XC // 128), (c + 1) * (XC // 128)):
            cp_out.append(copy(dxb.at[cc, :, 0:T], dx_h.at[:, :, lanes(cc)]))

    for cp in cp_out:
        cp.wait()


@jax.jit
def pallas_standalone__seq2seq_rnn_t_joint__speech_kernel(
    x: jax.Array, w1: jax.Array, w2: jax.Array, g: jax.Array,
    w_f: jax.Array, w_g: jax.Array, w_o: jax.Array, grad_out: jax.Array,
):
    assert x.shape == (B, T, D) and w1.shape == (5, D, D) and g.shape == (B, U, D)
    sds = lambda *s: jax.ShapeDtypeStruct(s, BF16)
    vm = pltpu.VMEM
    hbm = pl.BlockSpec(memory_space=pltpu.MemorySpace.HBM)
    out, dx, dw1, dw2, dg, dwf, dwg, dwo = pl.pallas_call(
        _kernel,
        in_specs=[hbm] * 8,
        out_specs=[hbm] * 8,
        out_shape=[sds(JR, D), sds(B, T, D), sds(5, D, D), sds(5, D, D), sds(B * U, D),
                   sds(D, D), sds(D, D), sds(D, D)],
        scratch_shapes=[
            vm((LC, B, XROWS, 128), BF16), vm((11 * D, D), BF16), vm((7 * D, D), BF16),
            vm((3, D, D), BF16), vm((B * U, D), BF16), vm((D, D), BF16), vm((D, D), BF16),
            vm((D, D), BF16), vm((JR, D), BF16),
            vm((JR, D), F32), vm((R, 11 * D), BF16), vm((R, 7 * D), BF16),
            vm((4, R, D), F32), vm((2, R, D), F32), vm((2 * R, D), BF16), vm((2 * R, D), F32),
            vm((JR, D), BF16), vm((2 * R, D), BF16), vm((4, R, D), BF16), vm((6, R, D), BF16),
            vm((JR, D), BF16), vm((LC, B, 8 * NP, 128), BF16), vm((5, D, D), BF16),
            vm((5, D, D), BF16), vm((B * U, D), BF16), vm((D, D), BF16), vm((D, D), BF16),
            vm((D, D), BF16), pltpu.SemaphoreType.DMA((64,)),
        ],
        compiler_params=pltpu.CompilerParams(
            vmem_limit_bytes=100 * 1024 * 1024, flags=CFG["flags"] or None),
    )(x, w1, w2, g.reshape(B * U, D), w_f, w_g, w_o, grad_out.reshape(JR, D))
    return (out.reshape(B, 2 * NT, U, D), dx, dw1, dw2, dg.reshape(B, U, D), dwf, dwg, dwo)
```

```python
import math
from functools import partial

import jax
import jax.numpy as jnp
from jax import lax
import jax.experimental.pallas as pl
import jax.experimental.pallas.tpu as pltpu

F32, BF16, I32 = jnp.float32, jnp.bfloat16, jnp.int32
B, T, D, U = 2, 1000, 512, 8
T1, T2 = T // 2, T // 4
NT = T2 // 2
JR = T2 * U
NP = 64
R = {1: 2 * B * NP, 2: B * NP}
H = D // 2
XROWS = 16 + 16 * NP + 16
LC = D // 128

CHUNKS = (8, 16, 24, 32, 16, 16, 13)
GROUPS = ((0, 1), (2,), (3,), (4,), (5, 6))
DWO_GROUPS = ((0, 2), (1, 3), (4, 5, 6))
LATE = (5, 6, 0)
LOAD_ORDER = "wo g0 g1 g2 g3 g4 x0 x1 a0 x2 x3 a1 b0 b1 g6 rest g5".split()
WS = 16

PA2, PB2 = 0.5, 2.0
PA, PB = math.sqrt(PA2), math.sqrt(PB2)
IA, IB = 1.0 / (2 * PA2 * (PA2 - PB2)), 1.0 / (2 * PB2 * (PB2 - PA2))
GC = math.sqrt(2.0 / math.pi)
GK = 0.044715


def _dot(a, b):
    return lax.dot_general(a, b, (((1,), (0,)), ((), ())), preferred_element_type=F32)


def _dot_nt(a, b):
    return lax.dot_general(a, b, (((1,), (1,)), ((), ())), preferred_element_type=F32)


def _dot_tn(a, b):
    return lax.dot_general(a, b, (((0,), (0,)), ((), ())), preferred_element_type=F32)


def _gelu(x):
    return x * (0.5 + 0.5 * jnp.tanh(x * (GC + (GC * GK) * (x * x))))


def _gelu_grad(x):
    x2 = x * x
    t = jnp.tanh(x * (GC + (GC * GK) * x2))
    cdf = 0.5 + 0.5 * t
    return cdf + (x * cdf) * (1.0 - t) * (GC + (3.0 * GC * GK) * x2)


def _prev(v, above=None):
    edge = jnp.zeros_like(v[:8]) if above is None else above[above.shape[0] - 8:]
    return pltpu.roll(jnp.concatenate([v, edge], axis=0), 1, 0)[:v.shape[0]]


def _next(v, below=None):
    edge = jnp.zeros_like(v[:8]) if below is None else below[:8]
    return pltpu.roll(jnp.concatenate([v, edge], axis=0), v.shape[0] + 7, 0)[:v.shape[0]]


def _mask_tail(v, j):
    n = v.shape[0] - 8
    keep = 8 * (lax.broadcasted_iota(I32, (8, v.shape[1]), 0) + NP - 8) + j < T1
    return jnp.concatenate([v[:n], jnp.where(keep, v[n:], 0.0)], axis=0)


def _to_points(d):
    res = [d[0] - (PA2 + PB2) * d[2] + d[4]]
    for p, q2 in ((PA, PB2), (PB, PA2)):
        ev, od = d[4] - q2 * d[2], p * (d[3] - q2 * d[1])
        res += [ev + od, ev - od]
    return res + ([d[1] - (PA2 + PB2) * d[3] + d[5]] if len(d) == 6 else [])


def _to_points_t(r):
    sa, da, sb, db = r[1] + r[2], r[1] - r[2], r[3] + r[4], r[3] - r[4]
    d1, d3 = (-PA * PB2) * da - (PB * PA2) * db, PA * da + PB * db
    if len(r) == 6:
        d1, d3 = d1 + r[5], d3 - (PA2 + PB2) * r[5]
    return [d1, (-(PA2 + PB2)) * r[0] - PB2 * sa - PA2 * sb, d3, r[0] + sa + sb]


def _from_points(m):
    sa, da, sb, db = m[1] + m[2], m[1] - m[2], m[3] + m[4], m[3] - m[4]
    return (m[0] + IA * sa + IB * sb, (IA * PA) * da + (IB * PB) * db,
            (IA * PA2) * sa + (IB * PB2) * sb,
            (IA * PA * PA2) * da + (IB * PB * PB2) * db + m[5])


def _from_points_t(dy):
    res = [dy[0]]
    for p, p2, inv in ((PA, PA2, IA), (PB, PB2, IB)):
        ev, od = inv * dy[0] + (inv * p2) * dy[2], (inv * p) * dy[1] + (inv * p * p2) * dy[3]
        res += [ev + od, ev - od]
    return res + [dy[3]]


def _bf16_bits(v):
    return lax.bitcast_convert_type(v.astype(BF16).astype(F32), I32)


def _fold(p, q, k):
    hi = (lax.broadcasted_iota(I32, p.shape, 0) & k) != 0
    return jnp.where(hi, q, p) + pltpu.roll(jnp.where(hi, p, q), k, 0)


def _mix(*queues):
    order = sorted((i / len(q), -k, i) for k, q in enumerate(queues) for i in range(len(q)))
    for _, k, i in order:
        queues[-k][i]()


def _get(ref, *idx, rows=None):
    rows = slice(None) if rows is None else slice(rows.start // 2, rows.stop // 2)
    return pltpu.bitcast(ref.bitcast(I32)[(*idx, rows)], BF16)


def _put(v, ref, *idx, rows=None):
    ref[(*idx, slice(None) if rows is None else rows)] = v.astype(BF16)


def _load(ref, idx, strips, rows=None):
    return jnp.concatenate([_get(ref, *idx, c, rows=rows) for c in strips], axis=1)


def _store(ref, idx, strips, v, rows=None):
    for n, c in enumerate(strips):
        _put(v[:, n * 128:(n + 1) * 128], ref, *idx, c, rows=rows)


def _part(i, n=128):
    return slice(i * n, (i + 1) * n)


def _scratch():
    def bf(*shape):
        return pltpu.VMEM(shape + (128,), BF16)

    def f32(*shape):
        return pltpu.VMEM(shape, F32)

    ch = [16 * n for n in CHUNKS]
    return dict(
        wo=bf(LC, D), wc=bf(7, 2, H), wf=bf(LC, D), wg=bf(LC, D), g=pltpu.VMEM((B * U, D), BF16),
        go=[bf(LC, B, n) for n in ch], gc=[bf(5, 2, n) for n in ch], jc=[bf(7, 2, n) for n in ch],
        dj=[f32(B, n, D) for n in ch],
        dz=f32(4 * B, 4 * NP, D), out=[bf(LC, B, n) for n in ch], qc=f32(7, H, H),
        x=bf(LC, B, XROWS), dx=bf(LC, B, 16 * NP),
        f=bf(LC, 4 * R[2]), fe=f32(4 * R[2], D), dfe=f32(4 * R[2], D),
        conv={n: dict(w=[bf(LC, 5, H)] * 2, wt=[bf(8, LC, H)] * 2, xt=bf(LC, 11, R[n]),
                      m=f32(LC, 6, R[n], 128), pre=f32(LC, 4, R[n], 128), dm=bf(6, LC, R[n]),
                      r=[f32(11, R[n], H)] * 2, dw=[bf(LC, 5, H)] * 2) for n in R},
        dg=pltpu.VMEM((B * U, D), BF16), dwf=bf(LC, D), dwg=bf(LC, D), dwo=bf(LC, D),
        sem=pltpu.SemaphoreType.DMA((56,)),
    )


def _kernel(x_h, w1_h, w2_h, g_h, wf_h, wg_h, wo_h, go_h,
            out_h, dx_h, dw1_h, dw2_h, dg_h, dwf_h, dwg_h, dwo_h, s):
    n_sem, stores = [0], []
    ALL, HALF = range(LC), (range(0, 2), range(2, 4))
    first = [sum(CHUNKS[:i]) for i in range(len(CHUNKS) + 1)]
    span = [slice(16 * lo, 16 * hi) for lo, hi in zip(first, first[1:])]

    def copy(src, dst):
        cp = pltpu.make_async_copy(src, dst, s["sem"].at[n_sem[0]])
        n_sem[0] += 1
        cp.start()
        return cp

    def strips(hbm, idx, buf, load):
        sem = s["sem"].at[n_sem[0]]
        n_sem[0] += 1
        for c in ALL:
            pair = (hbm.at[(*idx, _part(c))], buf.at[c])
            pltpu.make_async_copy(*(pair if load else pair[::-1]), sem).start()
        return [pltpu.make_async_copy(buf, buf, sem)]

    def fetch(hbm, idx, buf):
        return strips(hbm, idx, buf, True)

    def flush(buf, hbm, idx):
        stores.extend(strips(hbm, idx, buf, False))

    def wait(cps):
        for cp in cps:
            cp.wait()

    every = slice(None)
    loaders = dict(wo=lambda: fetch(wo_h, (every,), s["wo"]),
                   rest=lambda: fetch(wf_h, (every,), s["wf"]) + fetch(wg_h, (every,), s["wg"])
                   + [copy(g_h, s["g"])])
    for i in range(len(span)):
        loaders[f"g{i}"] = partial(fetch, go_h, (every, span[i]), s["go"][i])
    for k in range(2):
        loaders[f"a{k}"] = partial(fetch, w1_h, (every, _part(k, H)), s["conv"][1]["w"][k])
        loaders[f"b{k}"] = partial(fetch, w2_h, (every, _part(k, H)), s["conv"][2]["w"][k])
    for c in ALL:
        loaders[f"x{c}"] = lambda c=c: [copy(x_h.at[:, :, _part(c)], s["x"].at[c, :, 16:16 + T])]
    loads = {name: loaders[name]() for name in LOAD_ORDER}

    def need(names):
        for name in names.split():
            wait(loads.pop(name))

    def go_block(i, b, half):
        return jnp.concatenate([_get(s["go"][i], c, b) for c in HALF[half]], axis=1)

    def g_comb(r, i):
        return go_block(i, 6 - r, 6 - r) if r >= 5 else _load(s["gc"][i], (r,), range(2))

    def w_comb(r):
        if r in (1, 4):
            return _load(s["wo"], (), HALF[r // 4], _part(r // 4, H))
        return _load(s["wc"], (r,), range(2))

    def make_wc():
        w11, w12, w21, w22 = (_load(s["wo"], (), HALF[j], _part(i, H)).astype(F32)
                              for i in range(2) for j in range(2))
        for r, v in ((5, w11 + w12), (6, w21 + w22), (0, w11 + w22), (2, w12 - w22), (3, w21 - w11)):
            _store(s["wc"], (r,), range(2), v)

    def make_gc(i):
        n = span[i].stop - span[i].start
        for lo in range(0, n, 64):
            rows = slice(lo, min(lo + 64, n))
            for c in range(2):
                g11, g12, g21, g22 = (_get(s["go"][i], c + 2 * j, b, rows=rows).astype(F32)
                                      for b in range(B) for j in range(2))
                for r, v in enumerate((g11 + g22, g21 - g22, g12 + g22, g11 + g21, g12 - g11)):
                    _put(v, s["gc"][i], r, c, rows=rows)

    def steps(gen, n):
        return [partial(next, gen)] * n

    def joint_dj(i):
        def p(r):
            return _dot_nt(g_comb(r, i), w_comb(r))
        dj, n = s["dj"][i], span[i].stop - span[i].start
        p6 = p(5)
        yield p6
        p7 = p(6)
        make_gc(i)
        yield p7
        p5 = p(4)
        dj[0, :n, _part(1, H)] = (p5 + p7)
        d11 = p5 - p6
        yield p5
        p2 = p(1)
        dj[1, :n, _part(0, H)] = (p2 + p6)
        d22 = p2 - p7
        yield p2
        p1 = p(0)
        yield p1
        p3 = p(2)
        dj[0, :n, _part(0, H)] = (p3 + d11 + p1)
        yield p3
        p4 = p(3)
        dj[1, :n, _part(1, H)] = (p4 + d22 + p1)
        yield p4

    def joint_out(i):
        def m(r):
            return _dot(_load(s["jc"][i], (r,), range(2)), w_comb(r))

        def put(b, half, v):
            for n, c in enumerate(HALF[half]):
                s["out"][i][c, b] = v[:, _part(n)].astype(BF16)
        m5 = m(4)
        yield m5
        m2 = m(1)
        yield m2
        m3 = m(2)
        put(0, 1, m3 + m5)
        c22 = m3 - m2
        yield m3
        m4 = m(3)
        put(1, 0, m4 + m2)
        c11 = m4 - m5
        yield m4
        m1 = m(0)
        yield m1
        m7 = m(6)
        put(0, 0, m7 + c11 + m1)
        yield m7
        m6 = m(5)
        put(1, 1, m6 + c22 + m1)
        flush(s["out"][i], out_h, (every, span[i]))
        yield m6

    def joint_dwo(r, group):
        q = _dot_tn(jnp.concatenate([_load(s["jc"][i], (r,), range(2)) for i in group], axis=0),
                    jnp.concatenate([g_comb(r, i) for i in group], axis=0))
        s["qc"][r] = q if group[0] == 0 else s["qc"][r] + q
        return q

    def finish_dwo():
        q1, q2, q3, q4, q5, q6, q7 = (s["qc"][r] for r in range(7))
        for i, v in enumerate((q1 + q2 - q4 + q6, q3 + q6, q4 + q7, q1 - q3 + q5 + q7)):
            _store(s["dwo"], (), HALF[i % 2], v, _part(i // 2, H))
        flush(s["dwo"], dwo_h, (every,))

    dge = {}

    def joint_tanh(ge, i, m0, c):
        dz = {}
        for lo in range(m0, min(m0 + 4, NT), 2):
            n = min(2, NT - lo)
            rows = slice(16 * (lo - first[i]), 16 * (lo - first[i] + n))
            js = []
            for b in range(B):
                for cc in (c, c + 2):
                    j = jnp.concatenate(
                        [jnp.tanh(s["fe"][pl.ds((q * B + b) * NP + lo // 2, 1), _part(cc)]
                                  + ge[_part(b, U), _part(cc)]) for q in range(2 * n)], axis=0)
                    js.append(j)
                    v = s["dj"][i][b, rows, _part(cc)] * (1.0 - j * j)
                    v = [v[_part(q, U)] for q in range(2 * n)]
                    acc = sum(v[1:], v[0])
                    dge[b, cc] = dge[b, cc] + acc if (b, cc) in dge else acc
                    dz[b, cc] = dz.get((b, cc), []) + v
                    if lo > m0 or lo + n == NT:
                        v = dz[b, cc] + [jnp.zeros((U, 128), F32)] * (8 - len(dz[b, cc]))
                        for q in range(4):
                            s["dz"][q * B + b, _part(m0 // 4, U), _part(cc)] = _fold(v[q], v[4 + q], 1)
            a11, a12, a21, a22 = js
            for r, v in enumerate((a11 + a22, a21 + a22, a11, a22, a11 + a12, a21 - a11, a12 - a22)):
                _put(v, s["jc"][i], r, c, rows=rows)

    def joint_sums(qb, u):
        z = [s["dz"][qb, _part(4 * u + n, U)] for n in range(4)]
        s["dfe"][pl.ds(qb * NP + 8 * u, 8)] = _fold(_fold(z[0], z[1], 2), _fold(z[2], z[3], 2), 4)

    SLOTS = ((0, 1), (2, 3), (4, 5), (6, 7), (8, 9), (10,))
    RAW = {0: 0, 1: 1, 10: 4}
    cv = s["conv"]

    def x_point(n, k, p):
        return jnp.concatenate([_get(cv[n]["xt"], c, i) for i in SLOTS[p] for c in HALF[k]], axis=1)

    def w_point(n, k, p, strips):
        return jnp.concatenate(
            [jnp.concatenate([_get(cv[n]["w"][k], c, RAW[i]) if i in RAW
                              else _get(cv[n]["wt"][k], i - 2, c) for c in strips], axis=1)
             for i in SLOTS[p]], axis=0)

    def make_wt(n, k, c, u):
        g0, h0, g1, h1, g2 = (
            _get(cv[n]["w"][k], c, t, rows=_part(u, WS)).astype(F32) for t in range(5))
        for i, p, p2 in ((0, PA, PA2), (4, PB, PB2)):
            ev, od, oo = g0 + p2 * g2, p * g1, p * h1
            for m, v in enumerate((ev + od, h0 + oo, ev - od, h0 - oo)):
                _put(v, cv[n]["wt"][k], i + m, c, rows=_part(u, WS))

    def put_points(n, c, rows, even, odd):
        for ph, d in enumerate((even, odd)):
            for p, v in enumerate(_to_points(d)):
                _put(v, cv[n]["xt"], c, 2 * p + ph, rows=rows)

    def make_xt1(c, u):
        xw = s["x"].bitcast(I32)
        b, lo = divmod(u * WS, NP)
        if lo == 0:
            xw[c, b, 0:8] = jnp.zeros((8, 128), I32)
        if lo + WS == NP:
            tail = slice((16 + T) // 2 - 4, XROWS // 2)
            keep = lax.broadcasted_iota(I32, (tail.stop - tail.start, 128), 0) < 4
            xw[c, b, tail] = jnp.where(keep, xw[c, b, tail], 0)
        words = [xw[c, b, pl.ds(7 + k + 8 * lo, WS, stride=8), :] for k in range(10)]
        even = [lax.bitcast_convert_type(w << 16, F32) for w in words]
        odd = [lax.bitcast_convert_type(w & -65536, F32) for w in words[:9]]
        for e in range(2):
            put_points(1, c, _part(e * R[2] // WS + u, WS),
                       even[4 * e:4 * e + 6], odd[4 * e:4 * e + 5])

    def conv_dot(n, p, k, strips):
        v = _dot(x_point(n, k, p), w_point(n, k, p, strips))
        for i, c in enumerate(strips):
            cv[n]["m"][c, p] = v[:, _part(i)] + cv[n]["m"][c, p] if k else v[:, _part(i)]

    def activate(n, c, rows):
        pre = _from_points([cv[n]["m"][c, p, rows] for p in range(6)])
        for q in range(4):
            cv[n]["pre"][c, q, rows] = pre[q]
        return [_gelu(v) for v in pre]

    def finish_conv1(c, b):
        h = [_mask_tail(v, 4 * e + q) for e in range(2)
             for q, v in enumerate(activate(1, c, _part(e * B + b, NP)))]
        put_points(2, c, _part(b, NP), [_prev(h[6])] + h[0::2] + [_next(h[0])],
                   [_prev(h[7])] + h[1::2])

    def finish_conv2(c, u):
        for q, v in enumerate(activate(2, c, _part(u, WS))):
            _put(v, s["f"], c, rows=_part(q * R[2] // WS + u, WS))

    def back_activate(n, c, rows, grads, j0=None):
        dy = [g * _gelu_grad(cv[n]["pre"][c, q, rows]) for q, g in enumerate(grads)]
        if j0 is not None:
            dy = [_mask_tail(v, j0 + q) for q, v in enumerate(dy)]
        for p, v in enumerate(_from_points_t(dy)):
            _put(v, cv[n]["dm"], p, c, rows=rows)

    def back_dot(n, p, k):
        v = _dot_nt(_load(cv[n]["dm"], (p,), ALL), w_point(n, k, p, ALL))
        for m, i in enumerate(SLOTS[p]):
            cv[n]["r"][k][i] = v[:, _part(m, H)]

    def get_points(n, c, rows):
        return [[cv[n]["r"][c // 2][i, rows, _part(c % 2)] for i in range(ph, 11, 2)]
                for ph in range(2)]

    def conv2_dx(c, b):
        re, ro = get_points(2, c, _part(b, NP))
        de, do = _to_points_t(re), _to_points_t(ro)
        de[0], de[3], do[3] = de[0] + _prev(re[5]), de[3] + _next(re[0]), do[3] + _next(ro[0])
        for e in range(2):
            back_activate(1, c, _part(e * B + b, NP),
                          [de[2 * e], do[2 * e], de[2 * e + 1], do[2 * e + 1]], 4 * e)

    def conv1_dx(c, b):
        (re0, ro0), (re1, ro1) = (get_points(1, c, _part(e * B + b, NP)) for e in range(2))
        words = s["dx"].bitcast(I32)
        for e, (re, ro, before, after_e, after_o) in enumerate((
                (re0, ro0, _prev(re1[5]), re1[0], ro1[0]),
                (re1, ro1, re0[5], _next(re0[0]), _next(ro0[0])))):
            de, do = _to_points_t(re), _to_points_t(ro)
            de[0], de[3], do[3] = de[0] + before, de[3] + after_e, do[3] + after_o
            for q in range(4):
                words[c, b, pl.ds(4 * e + q, NP, stride=8), :] = (
                    lax.shift_right_logical(_bf16_bits(de[q]), 16) | _bf16_bits(do[q]))

    def conv_dw(n, k):
        def q(p):
            return _dot_tn(x_point(n, k, p), _load(cv[n]["dm"], (p,), ALL))

        def put(t, v):
            for ph in range(v.shape[0] // H):
                for c in ALL:
                    _put(v[_part(ph, H), _part(c)], cv[n]["dw"][k], c, t + ph)
        qa = q(1)
        yield
        qna = q(2)
        sa, da = qa + qna, PA * (qa - qna)
        yield
        qb = q(3)
        yield
        qnb = q(4)
        sb = qb + qnb
        put(2, da + PB * (qb - qnb))
        s0, s2 = sa + sb, PA2 * sa[:H] + PB2 * sb[:H]
        yield
        put(0, s0 + q(0))
        yield
        put(4, s2 + q(5))
        yield

    def per_strip(fn, k, count):
        return [partial(fn, c, u) for c in HALF[k] for u in range(count)]

    def weights(n, k):
        return [partial(make_wt, n, k, c, u) for c in ALL for u in range(H // WS)]

    def gelu1(c):
        return [partial(finish_conv1, c, b) for b in range(B)]

    def gelu2(c):
        return [partial(finish_conv2, c, u) for u in range(R[2] // WS)]

    def conv(n, k, strips, points):
        return [partial(conv_dot, n, p, k, strips) for p in points]

    def dj(ids):
        return [t for i in ids for t in steps(joint_dj(i), 7)]

    def outs(ids):
        return [t for i in ids for t in steps(joint_out(i), 7)]

    def paired(n, k, groups):
        return [t for points in groups for c in ALL for t in conv(n, k, (c,), points)]

    def tiles(fn, group, step):
        return [partial(fn, i, n0, c)
                for i in group for n0 in range(first[i], first[i + 1], step) for c in range(2)]

    need("wo g0")
    make_wc()
    _mix(dj([0]))
    for i in (1, 2, 3):
        need(f"g{i}")
        _mix(dj([i]))
    need("x0 x1 g4")
    _mix(dj([4]), per_strip(make_xt1, 0, R[2] // WS))
    need("a0")
    _mix(paired(1, 0, ((0,), (5,))), weights(1, 0))
    _mix(paired(1, 0, ((1, 2), (3, 4))))
    need("x2 x3 a1")
    _mix(per_strip(make_xt1, 1, R[2] // WS))
    _mix(paired(1, 1, ((0,), (5,))), weights(1, 1))
    _mix(paired(1, 1, ((1, 2),)))
    _mix(conv(1, 1, (0,), (3, 4)))
    _mix(conv(1, 1, (1,), (3, 4)), gelu1(0))
    need("b0 b1 g6")
    _mix(conv(1, 1, (2,), (3, 4)), gelu1(1))
    _mix(conv(1, 1, (3,), (3, 4)) + dj([6]), gelu1(2), weights(2, 0))
    _mix(paired(2, 0, ((0,), (5,), (1, 2), (3, 4))), gelu1(3), weights(2, 1))
    for c in ALL:
        _mix(conv(2, 1, (c,), range(6)), gelu2(c - 1) if c else [])
    need("rest g5")
    ge = _dot(s["g"][...], _load(s["wg"], (), ALL))
    filler = dj([5])
    _mix(filler[:3], gelu2(LC - 1))
    s["fe"][...] = _dot(_load(s["f"], (), ALL), _load(s["wf"], (), ALL))

    prev, sums, done = filler[3:], [], 0
    for group in GROUPS:
        _mix(prev, tiles(partial(joint_tanh, ge), group, 4), sums)
        prev = outs([i for i in group if i not in LATE])
        prev += [partial(joint_dwo, r, ids) for ids in DWO_GROUPS if ids[-1] in group
                 for r in range(7)]
        ready = (first[group[-1] + 1] + 3) // 16
        sums = [partial(joint_sums, qb, u) for u in range(done, ready) for qb in range(4 * B)]
        done = ready
    _mix(prev, sums)
    dfe = s["dfe"][...].astype(BF16)
    df = _dot_nt(dfe, _load(s["wf"], (), ALL))
    for c in ALL:
        back_activate(2, c, _part(0, R[2]), [df[_part(q, R[2]), _part(c)] for q in range(4)])
    dge_b = jnp.concatenate(
        [jnp.concatenate([dge[b, c] for c in ALL], axis=1) for b in range(B)],
        axis=0).astype(BF16)
    s["dg"][...] = _dot_nt(dge_b, _load(s["wg"], (), ALL)).astype(BF16)
    _store(s["dwg"], (), ALL, _dot_tn(s["g"][...], dge_b))
    _store(s["dwf"], (), ALL, _dot_tn(_load(s["f"], (), ALL), dfe))
    finish_dwo()
    stores.append(copy(s["dg"], dg_h))
    flush(s["dwg"], dwg_h, (every,))
    flush(s["dwf"], dwf_h, (every,))

    for k in range(2):
        _mix([partial(back_dot, 2, p, k) for p in range(6)], per_strip(conv2_dx, 0, B * k))
    _mix(steps(conv_dw(2, 0), 6) + steps(conv_dw(2, 1), 6), per_strip(conv2_dx, 1, B))
    for k in range(2):
        flush(cv[2]["dw"][k], dw2_h, (every, _part(k, H)))
    for k in range(2):
        _mix([partial(back_dot, 1, p, k) for p in range(6)], per_strip(conv1_dx, 0, B * k))
    def flush_dx(k):
        stores.extend(copy(s["dx"].at[c, :, 0:T], dx_h.at[:, :, _part(c)]) for c in HALF[k])

    early, late = steps(conv_dw(1, 0), 6), steps(conv_dw(1, 1), 6)
    _mix(early[:1])
    flush_dx(0)
    _mix(early[1:], per_strip(conv1_dx, 1, B))
    _mix(late[:1])
    flush_dx(1)
    flush(cv[1]["dw"][0], dw1_h, (every, _part(0, H)))
    wait([stores.pop(0)])
    _mix(late[1:])
    flush(cv[1]["dw"][1], dw1_h, (every, _part(1, H)))
    wait([stores.pop(0)])
    _mix(outs(LATE[:-1]))
    wait([stores.pop(0)])
    _mix(outs(LATE[-1:]))
    wait(stores)


@jax.jit
def pallas_standalone__seq2seq_rnn_t_joint__speech_kernel(
    x: jax.Array, w1: jax.Array, w2: jax.Array, g: jax.Array,
    w_f: jax.Array, w_g: jax.Array, w_o: jax.Array, grad_out: jax.Array,
):
    assert x.shape == (B, T, D) and w1.shape == (5, D, D) and g.shape == (B, U, D)
    sds = lambda *s: jax.ShapeDtypeStruct(s, BF16)
    hbm = pl.BlockSpec(memory_space=pltpu.MemorySpace.HBM)
    out, dx, dw1, dw2, dg, dwf, dwg, dwo = pl.pallas_call(
        _kernel,
        in_specs=[hbm] * 8,
        out_specs=[hbm] * 8,
        out_shape=[sds(B, JR, D), sds(B, T, D), sds(5, D, D), sds(5, D, D), sds(B * U, D),
                   sds(D, D), sds(D, D), sds(D, D)],
        scratch_shapes=[_scratch()],
        compiler_params=pltpu.CompilerParams(
            vmem_limit_bytes=100 * 1024 * 1024,
            disable_bounds_checks=True, disable_semaphore_checks=True),
    )(x, w1, w2, g.reshape(B * U, D), w_f, w_g, w_o, grad_out.reshape(B, JR, D))
    return (out.reshape(B, 2 * NT, U, D), dx, dw1, dw2, dg.reshape(B, U, D), dwf, dwg, dwo)
```
